```python
import jax
import jax.numpy as jnp

def _softmax(x, axis=-1):
    return jax.nn.softmax(x, axis=axis)
def _gelu(x):
    return jax.nn.gelu(x, approximate=True)
def _silu(x):
    return jax.nn.silu(x)
def _sigmoid(x):
    return jax.nn.sigmoid(x)
def _layernorm(x, axis=-1, eps=1e-5):
    m = jnp.mean(x, axis=axis, keepdims=True)
    v = jnp.var(x, axis=axis, keepdims=True)
    return (x - m) / jnp.sqrt(v + eps)
def _scatter_add(tgt, idx, src, axis=0):
    return tgt.at[idx].add(src)
def _segment_sum(src, seg, n):
    return jax.ops.segment_sum(src, seg, n)
class _Rng:
    def __init__(self, key):
        self._k = key
    def _next(self):
        self._k, sub = jax.random.split(self._k)
        return sub
    def normal(self, shape):
        return jax.random.normal(self._next(), shape, dtype=jnp.bfloat16)
    def randint(self, lo, hi, shape):
        return jax.random.randint(self._next(), shape, lo, hi, dtype=jnp.int32)
    def uniform(self, shape, lo=0.0, hi=1.0):
        return jax.random.uniform(self._next(), shape, jnp.bfloat16, lo, hi)
    def permutation(self, n):
        return jax.random.permutation(self._next(), n)


kernel_name = 'sequential_preLN__sliding_block_cached__glu_gated_swiglu__decode'

def setup_inputs():
    _rng = _Rng(jax.random.key(int.from_bytes(__import__("os").urandom(4), "little")))
    _w = (lambda a: (lambda t: t.astype(jnp.bfloat16) if jnp.issubdtype(t.dtype, jnp.floating) else t)(jnp.asarray(a)))
    def _A_setup():
        B, Sq, D = 1, 1, 640
        Hq, Hkv, Sk, Dh = 32, 32, 32768, 192
        assert Hq % Hkv == 0, (Hq, Hkv)
        return {
            "x": _w((lambda *s: _rng.normal(s) * 0.05)(B, Sq, D)),
            "k_cache": _w((lambda *s: _rng.normal(s) * 0.05)(B, Hkv, Sk, Dh)),
            "v_cache": _w((lambda *s: _rng.normal(s) * 0.05)(B, Hkv, Sk, Dh)),
            "wq": _w((lambda *s: _rng.normal(s) * 0.05)(D, Hq * Dh) * (D ** -0.5)),
            "wo": _w((lambda *s: _rng.normal(s) * 0.05)(Hq * Dh, D) * ((Hq * Dh) ** -0.5)),
        }
    _A_in = _A_setup()

    def _B_setup():
        B, S, D, F = 1, 1, 640, 1536
        return {
            "x": _w((lambda *s: _rng.normal(s) * 0.05)(B, S, D)),
            "w1": _w((lambda *s: _rng.normal(s) * 0.05)(D, F) * (2.0 / D) ** 0.5),
            "w3": _w((lambda *s: _rng.normal(s) * 0.05)(D, F) * (2.0 / D) ** 0.5),
            "w2": _w((lambda *s: _rng.normal(s) * 0.05)(F, D) * (2.0 / F) ** 0.5),
        }
    _B_in = _B_setup()

    return {
        "A_x": _A_in["x"],
        "A_k_cache": _A_in["k_cache"],
        "A_v_cache": _A_in["v_cache"],
        "A_wq": _A_in["wq"],
        "A_wo": _A_in["wo"],
        "B_x": _B_in["x"],
        "B_w1": _B_in["w1"],
        "B_w3": _B_in["w3"],
        "B_w2": _B_in["w2"],
    }

def reference(A_x, A_k_cache, A_v_cache, A_wq, A_wo, B_x, B_w1, B_w3, B_w2):
    def _A_ref(x, k_cache, v_cache, wq, wo):
        B, Sq, D = x.shape
        Hq, Dh = 32, 192
        Hkv, Sk = k_cache.shape[1], k_cache.shape[2]
        W = min(4096, max(256, Sk // 4))
        rep = Hq // Hkv
        q = (lambda x, *d: x.transpose(*d))((x @ wq).reshape(B, Sq, Hq, Dh), 0, 2, 1, 3)
        k = jnp.repeat(k_cache[:, :, Sk - W:, :], rep, axis=1)
        v = jnp.repeat(v_cache[:, :, Sk - W:, :], rep, axis=1)
        scores = jnp.einsum("bhqd,bhkd->bhqk", q, k) * (Dh ** -0.5)
        p = _softmax(scores, axis=-1)
        o = jnp.einsum("bhqk,bhkd->bhqd", p, v)
        return (lambda x, *d: x.transpose(*d))(o, 0, 2, 1, 3).reshape(B, Sq, Hq * Dh) @ wo

    def _B_ref(x, w1, w3, w2):
        gate = jnp.einsum("bsd,df->bsf", x, w1)
        up = jnp.einsum("bsd,df->bsf", x, w3)
        h = _silu(gate) * up
        out = jnp.einsum("bsf,fd->bsd", h, w2)
        return out

    x = A_x
    h = x + _A_ref(_layernorm(x, axis=-1), A_k_cache, A_v_cache, A_wq, A_wo)
    h2 = h + _B_ref(_layernorm(h, axis=-1), B_w1, B_w3, B_w2)
    return h2
```

```python
import functools

import jax
import jax.numpy as jnp
import jax.experimental.pallas as pl
import jax.experimental.pallas.tpu as pltpu

_EPS = 1e-5


def _layernorm_f32(x):
    m = jnp.mean(x, axis=-1, keepdims=True)
    c = x - m
    v = jnp.mean(c * c, axis=-1, keepdims=True)
    return c / jnp.sqrt(v + _EPS)


def _kernel(
    x_hbm, kt_hbm, vt_hbm, wq_hbm, wo_hbm, w1_hbm, w3_hbm, w2_hbm,
    o_ref,
    x_v, kbuf, vbuf, wq_v, wo_v, w1_v, w3_v, w2_v, q_s, o_s,
    ksem, vsem, wsem,
    *, n_chunks, rows, head_dim, win, win_start, nbuf,
):
    scale = head_dim ** -0.5

    def k_copy(c, slot):
        return pltpu.make_async_copy(
            kt_hbm.at[pl.ds(c * rows, rows), pl.ds(win_start, win)],
            kbuf.at[slot], ksem.at[slot])

    def v_copy(c, slot):
        return pltpu.make_async_copy(
            vt_hbm.at[pl.ds(c * rows, rows), pl.ds(win_start, win)],
            vbuf.at[slot], vsem.at[slot])

    x_copy = pltpu.make_async_copy(x_hbm, x_v, wsem.at[0])
    wq_copy = pltpu.make_async_copy(wq_hbm, wq_v, wsem.at[1])
    wo_copy = pltpu.make_async_copy(wo_hbm, wo_v, wsem.at[2])
    w1_copy = pltpu.make_async_copy(w1_hbm, w1_v, wsem.at[3])
    w3_copy = pltpu.make_async_copy(w3_hbm, w3_v, wsem.at[4])
    w2_copy = pltpu.make_async_copy(w2_hbm, w2_v, wsem.at[5])

    x_copy.start()
    wq_copy.start()
    for c in range(nbuf):
        k_copy(c, c).start()
        v_copy(c, c).start()
    wo_copy.start(priority=1)
    w1_copy.start(priority=1)
    w3_copy.start(priority=1)
    w2_copy.start(priority=1)

    x_copy.wait()
    x = x_v[...].astype(jnp.float32)
    xn = _layernorm_f32(x).astype(jnp.bfloat16)
    xn8 = jnp.broadcast_to(xn, (8, xn.shape[1]))
    wq_copy.wait()
    q = jnp.dot(xn8, wq_v[...], preferred_element_type=jnp.float32)

    row_id = jax.lax.broadcasted_iota(jnp.int32, (8, rows), 0)
    col_id = jax.lax.broadcasted_iota(jnp.int32, (8, rows), 1)
    diag = jnp.logical_and(col_id >= row_id * head_dim,
                           col_id < (row_id + 1) * head_dim)
    for c in range(n_chunks):
        q_s[c] = jnp.where(diag, q[:, c * rows:(c + 1) * rows], 0.0).astype(jnp.bfloat16)

    def step(c, carry):
        slot = c % nbuf
        k_copy(c, slot).wait()
        s = jnp.dot(q_s[c], kbuf[slot], preferred_element_type=jnp.float32)

        @pl.when(c + nbuf < n_chunks)
        def _():
            k_copy(c + nbuf, slot).start()

        s = s * scale
        m = jnp.max(s, axis=-1, keepdims=True)
        p = jnp.exp(s - m)
        l = jnp.sum(p, axis=-1, keepdims=True)
        v_copy(c, slot).wait()
        o = jax.lax.dot_general(
            p.astype(jnp.bfloat16), vbuf[slot], (((1,), (1,)), ((), ())),
            preferred_element_type=jnp.float32)

        @pl.when(c + nbuf < n_chunks)
        def _():
            v_copy(c + nbuf, slot).start()

        o_s[c] = jnp.where(diag, o / l, 0.0).astype(jnp.bfloat16)
        return carry

    jax.lax.fori_loop(0, n_chunks, step, 0)

    wo_copy.wait()
    acc = jnp.zeros((8, x.shape[1]), jnp.float32)
    for c in range(n_chunks):
        acc = acc + jnp.dot(o_s[c], wo_v[c * rows:(c + 1) * rows, :],
                            preferred_element_type=jnp.float32)
    attn = jnp.sum(acc, axis=0, keepdims=True)
    h = x + attn
    hn = _layernorm_f32(h).astype(jnp.bfloat16)
    hn8 = jnp.broadcast_to(hn, (8, hn.shape[1]))
    w1_copy.wait()
    gate = jnp.dot(hn8, w1_v[...], preferred_element_type=jnp.float32)
    w3_copy.wait()
    up = jnp.dot(hn8, w3_v[...], preferred_element_type=jnp.float32)
    act = (gate * jax.nn.sigmoid(gate) * up).astype(jnp.bfloat16)
    w2_copy.wait()
    ffn = jnp.dot(act, w2_v[...], preferred_element_type=jnp.float32)
    o_ref[...] = (h + ffn[0:1, :]).astype(o_ref.dtype)


@jax.jit
def pallas_sequential_preLN__sliding_block_cached__glu_gated_swiglu__decode_kernel(
    A_x: jax.Array,
    A_k_cache: jax.Array,
    A_v_cache: jax.Array,
    A_wq: jax.Array,
    A_wo: jax.Array,
    B_x: jax.Array,
    B_w1: jax.Array,
    B_w3: jax.Array,
    B_w2: jax.Array,
):
    B, Sq, D = A_x.shape
    _, H, Sk, Dh = A_k_cache.shape
    F = B_w1.shape[1]
    assert B == 1 and Sq == 1
    W = min(4096, max(256, Sk // 4))
    heads_per_chunk = 2
    rows = heads_per_chunk * Dh
    n_chunks = H // heads_per_chunk
    nbuf = 3

    kt = jnp.swapaxes(A_k_cache, 2, 3).reshape(H * Dh, Sk)
    vt = jnp.swapaxes(A_v_cache, 2, 3).reshape(H * Dh, Sk)
    x2 = A_x.reshape(1, D)

    kernel = functools.partial(
        _kernel, n_chunks=n_chunks, rows=rows, head_dim=Dh, win=W,
        win_start=Sk - W, nbuf=nbuf)
    bf16 = jnp.bfloat16
    out = pl.pallas_call(
        kernel,
        out_shape=jax.ShapeDtypeStruct((1, D), A_x.dtype),
        in_specs=[pl.BlockSpec(memory_space=pl.ANY)] * 8,
        out_specs=pl.BlockSpec(memory_space=pltpu.VMEM),
        scratch_shapes=[
            pltpu.VMEM((1, D), bf16),
            pltpu.VMEM((nbuf, rows, W), bf16),
            pltpu.VMEM((nbuf, rows, W), bf16),
            pltpu.VMEM((D, H * Dh), bf16),
            pltpu.VMEM((H * Dh, D), bf16),
            pltpu.VMEM((D, F), bf16),
            pltpu.VMEM((D, F), bf16),
            pltpu.VMEM((F, D), bf16),
            pltpu.VMEM((n_chunks, 8, rows), bf16),
            pltpu.VMEM((n_chunks, 8, rows), bf16),
            pltpu.SemaphoreType.DMA((nbuf,)),
            pltpu.SemaphoreType.DMA((nbuf,)),
            pltpu.SemaphoreType.DMA((6,)),
        ],
        compiler_params=pltpu.CompilerParams(vmem_limit_bytes=100 * 1024 * 1024),
    )(x2, kt, vt, A_wq, A_wo, B_w1, B_w3, B_w2)
    return out.reshape(B, Sq, D)
```

```python
import functools

import jax
import jax.numpy as jnp
import jax.experimental.pallas as pl
import jax.experimental.pallas.tpu as pltpu

_EPS = 1e-5
_T = 128
_RING = 4
_LAG = 12
_KP0 = 4
_KPAIRS = 2
_KCOLS = 1024
_BG = (2, 5, 8)
_TICK = (4, 5)
_QK_HI = 24
_PV_HI = 28
_W2_SPLIT = (1024, 384, 128)


def _layernorm_f32(x):
    m = jnp.mean(x, axis=-1, keepdims=True)
    c = x - m
    v = jnp.mean(c * c, axis=-1, keepdims=True)
    return c / jnp.sqrt(v + _EPS)


def _spread(n_items, hi):
    return [(t * hi) // n_items for t in range(n_items)]


def _aligned(v, m):
    return v if isinstance(v, int) else pl.multiple_of(v, m)


def _kernel(
    x_hbm, kt_hbm, vt_hbm, wq_hbm, wo_hbm, w1_hbm, w3_hbm, w2_hbm,
    o_ref,
    x_v, kv, wq_v, wo_v, w1_v, w3_v, w2_v, q_s, s_scr, p_scr, o_s,
    psem, ksem, wsem, w2sem,
    *, n_pairs, head_dim, win, win_start,
):
    T, RING, lag = _T, _RING, _LAG
    f32, bf16 = jnp.float32, jnp.bfloat16
    scale = head_dim ** -0.5
    rows = 2 * head_dim
    nb = rows // T
    d_model = wq_v.shape[0]
    ncol = win // T
    n_rb = n_pairs * nb
    n_kb = _KP0 * nb
    krows = rows * _KPAIRS
    kq = win // _KCOLS
    n_strips = ((n_pairs - _KP0) // _KPAIRS) * kq
    pad = (n_rb + RING) * T

    def vrow(rb):
        return _aligned((n_rb + rb % RING) * T, T)

    def k_piece(kb, i):
        r0 = _aligned(kb * T, T)
        return pltpu.make_async_copy(
            kt_hbm.at[pl.ds(r0, T), pl.ds(win_start + i * T, T)],
            kv.at[pl.ds(r0, T), pl.ds(i * T, T)], psem.at[kb % RING])

    def v_piece(rb, i):
        return pltpu.make_async_copy(
            vt_hbm.at[pl.ds(_aligned(rb * T, T), T), pl.ds(win_start + i * T, T)],
            kv.at[pl.ds(vrow(rb), T), pl.ds(i * T, T)], psem.at[(n_kb + rb) % RING])

    def block_wait(row0, sem_idx):
        dst = kv.at[pl.ds(row0, T), :]
        pltpu.make_async_copy(dst, dst, psem.at[sem_idx]).wait()

    def k_strip(i):
        g = i // kq
        r0 = _aligned(_KP0 * rows + g * krows, T)
        c0 = _aligned((i % kq) * _KCOLS, _KCOLS)
        return pltpu.make_async_copy(
            kt_hbm.at[pl.ds(r0, krows), pl.ds(win_start + c0, _KCOLS)],
            kv.at[pl.ds(r0, krows), pl.ds(c0, _KCOLS)], ksem.at[g])

    x_copy = pltpu.make_async_copy(x_hbm, x_v, wsem.at[0])
    wq_copy = pltpu.make_async_copy(wq_hbm, wq_v, wsem.at[1])
    wo_copy = pltpu.make_async_copy(wo_hbm, wo_v, wsem.at[2])
    w1_copy = pltpu.make_async_copy(w1_hbm, w1_v, wsem.at[3])
    w3_copy = pltpu.make_async_copy(w3_hbm, w3_v, wsem.at[4])
    offs = [0]
    for s in _W2_SPLIT:
        offs.append(offs[-1] + s)
    w2_copies = [
        pltpu.make_async_copy(w2_hbm.at[pl.ds(offs[i], n), :],
                              w2_v.at[pl.ds(offs[i], n), :], w2sem.at[i])
        for i, n in enumerate(_W2_SPLIT)]
    tail = [wo_copy, w1_copy, w3_copy] + w2_copies

    def bg_count(p):
        return _BG[0] + ((p + 1) * _BG[1]) // _BG[2]

    assert _BG[1] <= _BG[2] and bg_count(n_kb + n_rb - 8) >= n_strips + len(tail)
    for c in range(_KP0, n_pairs, _KPAIRS):
        assert bg_count(n_kb + c * nb - 1) >= ((c - _KP0) // _KPAIRS + 1) * kq

    def bg_slot(p):
        i = bg_count(p - 1)
        new = bg_count(p) > i

        @pl.when(jnp.logical_and(new, i < n_strips))
        def _():
            k_strip(i).start(priority=1)

        for j, cp in enumerate(tail):
            @pl.when(jnp.logical_and(new, i == n_strips + j))
            def _():
                cp.start(priority=1)

    def tick():
        t = kv[pad:pad + 16, 0:T].astype(f32)[0:8]
        for _ in range(_TICK[0]):
            t = jax.lax.rsqrt(t + 1.0)
        for e in range(_TICK[1]):
            t = t * 0.5 if e % 2 == 0 else t + 0.25
        kv[pad:pad + 16, 0:T] = jnp.concatenate([t, t], axis=0).astype(bf16)

    def slots(lo, hi, start_fn, items):
        for i in range(lo, hi):
            start_fn(i + lag)
            for item in items.get(i, []):
                item()
            tick()

    wq_copy.start(priority=1)
    k_piece(0, 0).start()
    x_copy.start()
    kv[pad:pad + 16, 0:T] = jnp.zeros((16, T), bf16)

    def issue_strip(i, carry):
        k_strip(i).start(priority=1)
        return carry

    jax.lax.fori_loop(0, _BG[0], issue_strip, 0)
    for i in range(1, lag):
        k_piece(0, i).start()
        tick()

    row_id = jax.lax.broadcasted_iota(jnp.int32, (8, rows), 0)
    col_id = jax.lax.broadcasted_iota(jnp.int32, (8, rows), 1)
    diag = jnp.logical_and(col_id >= row_id * head_dim,
                           col_id < (row_id + 1) * head_dim)

    def k_period(kb, carry):
        bg_slot(kb)

        @pl.when(kb > 0)
        def _():
            block_wait(_aligned((kb - 1) * T, T), (kb - 1) % RING)

        slots(0, ncol, lambda i: k_piece(kb + i // ncol, i % ncol).start(), {})
        return carry

    jax.lax.fori_loop(0, n_kb - 1, k_period, 0)

    kb_last = n_kb - 1
    bg_slot(kb_last)
    block_wait((kb_last - 1) * T, (kb_last - 1) % RING)
    x_copy.wait()
    wq_copy.wait()
    x = x_v[...].astype(f32)
    xn8 = jnp.broadcast_to(_layernorm_f32(x).astype(bf16), (8, d_model))

    def q_compute(c):
        q = jnp.dot(xn8, wq_v[:, pl.ds(_aligned(c * rows, T), rows)],
                    preferred_element_type=f32)
        q_s[...] = jnp.where(diag, q, 0.0).astype(bf16)

    slots(0, ncol,
          lambda i: (k_piece(kb_last, i) if i < ncol else v_piece(0, i - ncol)).start(),
          {4: [lambda: q_compute(0)]})

    nt_dims = (((1,), (1,)), ((), ()))

    def o_block(k, o, linv):
        return jnp.where(diag[:, k * T:(k + 1) * T], o * linv, 0.0).astype(bf16)

    def pair_body(c, linv_prev):
        st = {}

        def pv_items(items, rb, k, pslot, get_linv, hi):
            for i, slot in enumerate(_spread(ncol, hi)):
                def item(i=i):
                    o = jax.lax.dot_general(
                        p_scr[pslot, :, i * T:(i + 1) * T],
                        kv[pl.ds(vrow(rb + RING), T), i * T:(i + 1) * T],
                        nt_dims, preferred_element_type=f32)
                    st["o"] = o if i == 0 else o + st["o"]
                    if i == ncol - 1:
                        o_s[rb + 1] = o_block(k, st["o"], get_linv())
                items.setdefault(slot, []).append(item)

        def qk_items(items):
            for i, slot in enumerate(_spread(ncol, _QK_HI)):
                def item(i=i):
                    r0 = pl.multiple_of(c * rows, T)
                    s = jnp.dot(q_s[...], kv[pl.ds(r0, rows), i * T:(i + 1) * T],
                                preferred_element_type=f32)
                    s_scr[:, i * T:(i + 1) * T] = s
                    st["m"] = s if i == 0 else jnp.maximum(st["m"], s)
                items.setdefault(slot, []).append(item)

            def softmax():
                m = jnp.max(st["m"], axis=-1, keepdims=True)
                p = jnp.exp((s_scr[...] - m) * scale)
                st["linv"] = 1.0 / jnp.sum(p, axis=-1, keepdims=True)
                p_scr[c % 2] = p.astype(bf16)
            items.setdefault(_QK_HI, []).append(softmax)

        for k in range(nb):
            rb = c * nb + k
            bg_slot(n_kb + rb)
            prev_sem = (n_kb + rb + RING - 1) % RING
            if k == 0:
                prev_row = jnp.where(c == 0, kb_last * T, vrow(rb + RING - 1))
                block_wait(pl.multiple_of(prev_row, T), prev_sem)

                @pl.when(jnp.logical_and(c >= _KP0, (c - _KP0) % _KPAIRS == 0))
                def _():
                    for j in range(kq):
                        k_strip(((c - _KP0) // _KPAIRS) * kq + j).wait()
            else:
                block_wait(vrow(rb - 1), prev_sem)

            def start_fn(i, rb=rb):
                v_piece(rb + i // ncol, i % ncol).start()

            items = {}
            if k == 0:
                pv_items(items, rb - 1, nb - 1, (c + 1) % 2, lambda: linv_prev, _PV_HI)
                qk_items(items)
                slots(0, ncol, start_fn, items)
            elif k < nb - 1:
                pv_items(items, rb - 1, k - 1, c % 2, lambda: st["linv"], _PV_HI)
                slots(0, ncol, start_fn, items)
            else:
                pv_items(items, rb - 1, k - 1, c % 2, lambda: st["linv"], ncol - lag - 2)
                slots(0, ncol - lag, start_fn, items)

                @pl.when(c < n_pairs - 1)
                def _():
                    slots(ncol - lag, ncol, start_fn,
                          {ncol - lag: [lambda: q_compute(c + 1)]})
        return st["linv"]

    linv = jax.lax.fori_loop(0, n_pairs, pair_body, jnp.ones((8, 1), f32))

    rb = n_rb - 1
    wo_copy.wait()
    acc = jnp.zeros((8, d_model), f32)
    for b in range(rb):
        acc = acc + jnp.dot(o_s[b + 1], wo_v[b * T:(b + 1) * T, :],
                            preferred_element_type=f32)
    block_wait(vrow(rb), (n_kb + rb) % RING)
    o = jax.lax.dot_general(p_scr[(n_pairs - 1) % 2], kv[pl.ds(vrow(rb), T), :],
                            nt_dims, preferred_element_type=f32)
    acc = acc + jnp.dot(o_block(nb - 1, o, linv), wo_v[rb * T:(rb + 1) * T, :],
                        preferred_element_type=f32)
    h = x + jnp.sum(acc, axis=0, keepdims=True)

    hn8 = jnp.broadcast_to(_layernorm_f32(h).astype(bf16), (8, d_model))
    w1_copy.wait()
    gate = jnp.dot(hn8, w1_v[...], preferred_element_type=f32)
    w3_copy.wait()
    up = jnp.dot(hn8, w3_v[...], preferred_element_type=f32)
    act = (gate * jax.nn.sigmoid(gate) * up).astype(bf16)
    n_last = _W2_SPLIT[-1]
    col = jnp.broadcast_to(act[0:1, offs[-1] - T:].astype(f32), (T, T)).T[T - n_last:, :]
    res = jnp.broadcast_to(h, (8, d_model))
    for i in range(len(w2_copies) - 1):
        w2_copies[i].wait()
        res = res + jnp.dot(act[:, offs[i]:offs[i + 1]], w2_v[offs[i]:offs[i + 1], :],
                            preferred_element_type=f32)
    w2_copies[-1].wait()
    w_last = w2_v[offs[-2]:offs[-1], :].astype(f32)
    prod = w_last * jnp.concatenate([col] * (d_model // T), axis=1)
    o_ref[...] = (res[0:1, :] + jnp.sum(prod, axis=0, keepdims=True)).astype(o_ref.dtype)


@jax.jit
def pallas_sequential_preLN__sliding_block_cached__glu_gated_swiglu__decode_kernel(
    A_x: jax.Array,
    A_k_cache: jax.Array,
    A_v_cache: jax.Array,
    A_wq: jax.Array,
    A_wo: jax.Array,
    B_x: jax.Array,
    B_w1: jax.Array,
    B_w3: jax.Array,
    B_w2: jax.Array,
):
    B, Sq, D = A_x.shape
    _, H, Sk, Dh = A_k_cache.shape
    F = B_w1.shape[1]
    W = min(4096, max(256, Sk // 4))
    assert B == 1 and Sq == 1 and H % 2 == 0 and (2 * Dh) % _T == 0
    assert sum(_W2_SPLIT) == F and W % _KCOLS == 0 and (Sk - W) % _T == 0
    n_pairs = H // 2
    assert (n_pairs - _KP0) % _KPAIRS == 0

    kt = jnp.swapaxes(A_k_cache, 2, 3).reshape(H * Dh, Sk)
    vt = jnp.swapaxes(A_v_cache, 2, 3).reshape(H * Dh, Sk)
    x2 = A_x.reshape(1, D)

    params = dict(vmem_limit_bytes=100 * 1024 * 1024)
    for name in ("disable_semaphore_checks", "disable_bounds_checks"):
        if hasattr(pltpu.CompilerParams, name):
            params[name] = True

    bf16 = jnp.bfloat16
    out = pl.pallas_call(
        functools.partial(_kernel, n_pairs=n_pairs, head_dim=Dh, win=W,
                          win_start=Sk - W),
        out_shape=jax.ShapeDtypeStruct((1, D), A_x.dtype),
        in_specs=[pl.BlockSpec(memory_space=pl.ANY)] * 8,
        out_specs=pl.BlockSpec(memory_space=pltpu.VMEM),
        scratch_shapes=[
            pltpu.VMEM((1, D), bf16),
            pltpu.VMEM((H * Dh + _RING * _T + 16, W), bf16),
            pltpu.VMEM((D, H * Dh), bf16),
            pltpu.VMEM((H * Dh, D), bf16),
            pltpu.VMEM((D, F), bf16),
            pltpu.VMEM((D, F), bf16),
            pltpu.VMEM((F, D), bf16),
            pltpu.VMEM((8, 2 * Dh), bf16),
            pltpu.VMEM((8, W), jnp.float32),
            pltpu.VMEM((2, 8, W), bf16),
            pltpu.VMEM((H * Dh // _T + 1, 8, _T), bf16),
            pltpu.SemaphoreType.DMA((_RING,)),
            pltpu.SemaphoreType.DMA(((n_pairs - _KP0) // _KPAIRS,)),
            pltpu.SemaphoreType.DMA((5,)),
            pltpu.SemaphoreType.DMA((len(_W2_SPLIT),)),
        ],
        compiler_params=pltpu.CompilerParams(**params),
    )(x2, kt, vt, A_wq, A_wo, B_w1, B_w3, B_w2)
    return out.reshape(B, Sq, D)
```

```python
import functools

import jax
import jax.numpy as jnp
import jax.experimental.pallas as pl
import jax.experimental.pallas.tpu as pltpu

_EPS = 1e-5
_T = 128
_RING = 4
_LAG = 18
_K_TICKS = 28
_V_TICKS = 27
_DEP_LAG = 4
_QK_SPLIT = (10, 24)
_QK_HI = 20
_PV_HI = 28
_WO_AT = 8
_W2_SPLIT = (1024, 384, 128)


def _layernorm_f32(x):
    m = jnp.mean(x, axis=-1, keepdims=True)
    c = x - m
    v = jnp.mean(c * c, axis=-1, keepdims=True)
    return c / jnp.sqrt(v + _EPS)


def _spread(n_items, lo, hi):
    return [lo + (t * (hi - lo)) // n_items for t in range(n_items)]


def _aligned(v, m):
    return v if isinstance(v, int) else pl.multiple_of(v, m)


def _kernel(
    x_hbm, kt_hbm, vt_hbm, wq_hbm, wo_hbm, w1_hbm, w3_hbm, w2_hbm,
    o_ref,
    x_v, kv, wq_v, wo_v, w1_v, w3_v, w2_v, q_s, s_scr, p_scr, o_s,
    psem, wsem,
    *, n_pairs, head_dim, win, win_start,
):
    T, RING, lag = _T, _RING, _LAG
    f32, bf16 = jnp.float32, jnp.bfloat16
    scale = head_dim ** -0.5
    rows = 2 * head_dim
    nb = rows // T
    d_model = wq_v.shape[0]
    ncol = win // T
    n_rb = n_pairs * nb
    pad = (n_rb + RING) * T
    qa, qb = _QK_SPLIT

    def vrow(rb):
        return _aligned((n_rb + rb % RING) * T, T)

    def k_piece(kb, i):
        r0 = _aligned(kb * T, T)
        return pltpu.make_async_copy(
            kt_hbm.at[pl.ds(r0, T), pl.ds(win_start + i * T, T)],
            kv.at[pl.ds(r0, T), pl.ds(i * T, T)], psem.at[kb % RING])

    def v_piece(rb, i):
        return pltpu.make_async_copy(
            vt_hbm.at[pl.ds(_aligned(rb * T, T), T), pl.ds(win_start + i * T, T)],
            kv.at[pl.ds(vrow(rb), T), pl.ds(i * T, T)], psem.at[(n_rb + rb) % RING])

    def block_wait(row0, sem_idx):
        dst = kv.at[pl.ds(row0, T), :]
        pltpu.make_async_copy(dst, dst, psem.at[sem_idx]).wait()

    x_copy = pltpu.make_async_copy(x_hbm, x_v, wsem.at[0])
    wq_copy = pltpu.make_async_copy(wq_hbm, wq_v, wsem.at[1])
    wo_copy = pltpu.make_async_copy(wo_hbm, wo_v, wsem.at[2])
    w1_copy = pltpu.make_async_copy(w1_hbm, w1_v, wsem.at[3])
    w3_copy = pltpu.make_async_copy(w3_hbm, w3_v, wsem.at[4])
    offs = [0]
    for n in _W2_SPLIT:
        offs.append(offs[-1] + n)
    w2_copies = [
        pltpu.make_async_copy(w2_hbm.at[pl.ds(offs[i], n), :],
                              w2_v.at[pl.ds(offs[i], n), :], wsem.at[5 + i])
        for i, n in enumerate(_W2_SPLIT)]
    late_copies = [w1_copy, w3_copy] + w2_copies

    def slots(lo, hi, start_fn, items, ticks):
        deps = {}
        for i in range(lo, hi):
            start_fn(i + lag)
            t = kv[pad:pad + 16, 0:T].astype(f32)[0:8]
            n_ops = ticks
            if i in deps:
                t = t + functools.reduce(lambda a, b: a + b, deps[i])
                n_ops -= 1
            for e in range(n_ops):
                t = t * 0.5 if e % 2 == 0 else t + 0.25
            for item in items.get(i, []):
                r = item()
                if r is not None:
                    deps.setdefault(i + _DEP_LAG, []).append(r)
            kv[pad:pad + 16, 0:T] = jnp.concatenate([t, t], axis=0).astype(bf16)

    wq_copy.start(priority=1)
    x_copy.start()
    kv[pad:pad + 16, 0:T] = jnp.zeros((16, T), bf16)
    slots(-lag, 0, lambda i: k_piece(0, i).start(), {}, _K_TICKS)

    def k_period(kb, carry):
        @pl.when(kb == _WO_AT)
        def _():
            wo_copy.start(priority=1)

        @pl.when(kb > 0)
        def _():
            block_wait(_aligned((kb - 1) * T, T), (kb - 1) % RING)

        slots(0, ncol, lambda i: k_piece(kb + i // ncol, i % ncol).start(), {}, _K_TICKS)
        return carry

    jax.lax.fori_loop(0, n_rb - 2, k_period, 0)

    row_id = jax.lax.broadcasted_iota(jnp.int32, (8, rows), 0)
    col_id = jax.lax.broadcasted_iota(jnp.int32, (8, rows), 1)
    diag = jnp.logical_and(col_id >= row_id * head_dim,
                           col_id < (row_id + 1) * head_dim)

    block_wait((n_rb - 3) * T, (n_rb - 3) % RING)
    x_copy.wait()
    wq_copy.wait()
    x = x_v[...].astype(f32)
    xn8 = jnp.broadcast_to(_layernorm_f32(x).astype(bf16), (8, d_model))

    def q_compute(c):
        q = jnp.dot(xn8, wq_v[:, pl.ds(_aligned(c * rows, T), rows)],
                    preferred_element_type=f32)
        q_s[...] = jnp.where(diag, q, 0.0).astype(bf16)

    def qk_items(items, c, cols, lo, hi):
        for i, slot in zip(cols, _spread(len(cols), lo, hi)):
            def item(i=i):
                s = jnp.dot(
                    q_s[...], kv[pl.ds(_aligned(c * rows, T), rows), i * T:(i + 1) * T],
                    preferred_element_type=f32)
                s_scr[:, i * T:(i + 1) * T] = s
                return s
            items.setdefault(slot, []).append(item)

    items = {4: [lambda: q_compute(0)]}
    qk_items(items, 0, range(0, qa), 12, ncol - 1)
    slots(0, ncol, lambda i: k_piece(n_rb - 2 + i // ncol, i % ncol).start(),
          items, _K_TICKS)

    block_wait((n_rb - 2) * T, (n_rb - 2) % RING)
    items = {}
    qk_items(items, 0, range(qa, qb), 0, ncol - 1)
    slots(0, ncol,
          lambda i: (k_piece(n_rb - 1, i) if i < ncol else v_piece(0, i - ncol)).start(),
          items, _K_TICKS)

    nt_dims = (((1,), (1,)), ((), ()))

    def o_block(k, o, linv):
        return jnp.where(diag[:, k * T:(k + 1) * T], o * linv, 0.0).astype(bf16)

    def pair_body(c, linv_prev):
        st = {}
        c_next = jnp.minimum(c + 1, n_pairs - 1)

        def pv_items(items, rb, k, pslot, get_linv, hi):
            for i, slot in enumerate(_spread(ncol, 0, hi)):
                def item(i=i):
                    o = jax.lax.dot_general(
                        p_scr[pslot, :, i * T:(i + 1) * T],
                        kv[pl.ds(vrow(rb + RING), T), i * T:(i + 1) * T],
                        nt_dims, preferred_element_type=f32)
                    st["o"] = o if i == 0 else o + st["o"]
                    if i == ncol - 1:
                        o_s[rb + 1] = o_block(k, st["o"], get_linv())
                    return o
                items.setdefault(slot, []).append(item)

        def softmax():
            s = s_scr[...]
            m = jnp.max(s, axis=-1, keepdims=True)
            p = jnp.exp((s - m) * scale)
            st["linv"] = 1.0 / jnp.sum(p, axis=-1, keepdims=True)
            p_scr[c % 2] = p.astype(bf16)

        for j, cp in enumerate(late_copies):
            @pl.when(c == j)
            def _():
                cp.start(priority=1)

        for k in range(nb):
            rb = c * nb + k
            prev_row = vrow(rb + RING - 1)
            if k == 0:
                prev_row = pl.multiple_of(jnp.where(c == 0, (n_rb - 1) * T, prev_row), T)
            block_wait(prev_row, (n_rb + rb + RING - 1) % RING)

            def start_fn(i, rb=rb):
                v_piece(rb + i // ncol, i % ncol).start()

            items = {}
            if k == 0:
                pv_items(items, rb - 1, nb - 1, (c + 1) % 2, lambda: linv_prev, _PV_HI)
                qk_items(items, c, range(qb, ncol), 0, _QK_HI)
                items.setdefault(_QK_HI + 1, []).append(softmax)
                slots(0, ncol, start_fn, items, _V_TICKS)
            elif k < nb - 1:
                items[0] = [lambda: q_compute(c_next)]
                pv_items(items, rb - 1, k - 1, c % 2, lambda: st["linv"], _PV_HI)
                qk_items(items, c_next, range(0, qa), 8, ncol - 1)
                slots(0, ncol, start_fn, items, _V_TICKS)
            else:
                pv_items(items, rb - 1, k - 1, c % 2, lambda: st["linv"], ncol - lag - 2)
                slots(0, ncol - lag, start_fn, items, _V_TICKS)

                @pl.when(c < n_pairs - 1)
                def _():
                    items = {}
                    qk_items(items, c + 1, range(qa, qb), ncol - lag, ncol - 1)
                    slots(ncol - lag, ncol, start_fn, items, _V_TICKS)
        return st["linv"]

    linv = jax.lax.fori_loop(0, n_pairs, pair_body, jnp.ones((8, 1), f32))

    rb = n_rb - 1
    wo_copy.wait()
    acc = jnp.zeros((8, d_model), f32)
    for b in range(rb):
        acc = acc + jnp.dot(o_s[b + 1], wo_v[b * T:(b + 1) * T, :],
                            preferred_element_type=f32)
    block_wait(vrow(rb), (n_rb + rb) % RING)
    o = jax.lax.dot_general(p_scr[(n_pairs - 1) % 2], kv[pl.ds(vrow(rb), T), :],
                            nt_dims, preferred_element_type=f32)
    acc = acc + jnp.dot(o_block(nb - 1, o, linv), wo_v[rb * T:(rb + 1) * T, :],
                        preferred_element_type=f32)
    h = x + jnp.sum(acc, axis=0, keepdims=True)

    hn8 = jnp.broadcast_to(_layernorm_f32(h).astype(bf16), (8, d_model))
    w1_copy.wait()
    gate = jnp.dot(hn8, w1_v[...], preferred_element_type=f32)
    w3_copy.wait()
    up = jnp.dot(hn8, w3_v[...], preferred_element_type=f32)
    act = (gate * jax.nn.sigmoid(gate) * up).astype(bf16)
    n_last = _W2_SPLIT[-1]
    col = jnp.broadcast_to(act[0:1, offs[-1] - T:].astype(f32), (T, T)).T[T - n_last:, :]
    res = jnp.broadcast_to(h, (8, d_model))
    for i in range(len(w2_copies) - 1):
        w2_copies[i].wait()
        res = res + jnp.dot(act[:, offs[i]:offs[i + 1]], w2_v[offs[i]:offs[i + 1], :],
                            preferred_element_type=f32)
    w2_copies[-1].wait()
    w_last = w2_v[offs[-2]:offs[-1], :].astype(f32)
    prod = w_last * jnp.concatenate([col] * (d_model // T), axis=1)
    o_ref[...] = (res[0:1, :] + jnp.sum(prod, axis=0, keepdims=True)).astype(o_ref.dtype)


@jax.jit
def pallas_sequential_preLN__sliding_block_cached__glu_gated_swiglu__decode_kernel(
    A_x: jax.Array,
    A_k_cache: jax.Array,
    A_v_cache: jax.Array,
    A_wq: jax.Array,
    A_wo: jax.Array,
    B_x: jax.Array,
    B_w1: jax.Array,
    B_w3: jax.Array,
    B_w2: jax.Array,
):
    B, Sq, D = A_x.shape
    _, H, Sk, Dh = A_k_cache.shape
    F = B_w1.shape[1]
    W = min(4096, max(256, Sk // 4))
    assert B == 1 and Sq == 1 and H % 2 == 0 and 2 * Dh == 3 * _T
    assert sum(_W2_SPLIT) == F and W == 32 * _T and (Sk - W) % _T == 0

    kt = jnp.swapaxes(A_k_cache, 2, 3).reshape(H * Dh, Sk)
    vt = jnp.swapaxes(A_v_cache, 2, 3).reshape(H * Dh, Sk)
    x2 = A_x.reshape(1, D)

    params = dict(vmem_limit_bytes=100 * 1024 * 1024)
    for name in ("disable_semaphore_checks", "disable_bounds_checks"):
        if hasattr(pltpu.CompilerParams, name):
            params[name] = True

    bf16 = jnp.bfloat16
    out = pl.pallas_call(
        functools.partial(_kernel, n_pairs=H // 2, head_dim=Dh, win=W, win_start=Sk - W),
        out_shape=jax.ShapeDtypeStruct((1, D), A_x.dtype),
        in_specs=[pl.BlockSpec(memory_space=pl.ANY)] * 8,
        out_specs=pl.BlockSpec(memory_space=pltpu.VMEM),
        scratch_shapes=[
            pltpu.VMEM((1, D), bf16),
            pltpu.VMEM((H * Dh + _RING * _T + 16, W), bf16),
            pltpu.VMEM((D, H * Dh), bf16),
            pltpu.VMEM((H * Dh, D), bf16),
            pltpu.VMEM((D, F), bf16),
            pltpu.VMEM((D, F), bf16),
            pltpu.VMEM((F, D), bf16),
            pltpu.VMEM((8, 2 * Dh), bf16),
            pltpu.VMEM((8, W), jnp.float32),
            pltpu.VMEM((2, 8, W), bf16),
            pltpu.VMEM((H * Dh // _T + 1, 8, _T), bf16),
            pltpu.SemaphoreType.DMA((_RING,)),
            pltpu.SemaphoreType.DMA((5 + len(_W2_SPLIT),)),
        ],
        compiler_params=pltpu.CompilerParams(**params),
    )(x2, kt, vt, A_wq, A_wo, B_w1, B_w3, B_w2)
    return out.reshape(B, Sq, D)
```

```python
import functools

import jax
import jax.numpy as jnp
import jax.experimental.pallas as pl
import jax.experimental.pallas.tpu as pltpu

_EPS = 1e-5
_T = 128
_GROUPS = 4
_LAG = 18
_K_TICKS = 28
_V_TICKS = 29
_DEP_LAG = 4
_QK_SPLIT = (6, 15, 24)
_QK_HI = 13
_MXU_HI = 21
_Q_SLOTS = 9
_HEAD_TILES = 3
_WO_AT = 8
_W2_SPLIT = (1024, 384, 128)


def _layernorm_f32(x):
    m = jnp.mean(x, axis=-1, keepdims=True)
    c = x - m
    v = jnp.mean(c * c, axis=-1, keepdims=True)
    return c / jnp.sqrt(v + _EPS)


def _spread(n_items, lo, hi):
    return [lo + (t * (hi - lo)) // n_items for t in range(n_items)]


def _aligned(v, m):
    return v if isinstance(v, int) else pl.multiple_of(v, m)


def _kernel(
    x_hbm, kt_hbm, vt_hbm, wq_hbm, wo_hbm, w1_hbm, w3_hbm, w2_hbm,
    o_ref,
    x_v, kbuf, vbuf, wq_v, wo_v, w1_v, w3_v, w2_v, xn_s, q_s, s_scr, p_scr, oacc, o_s,
    psem, wsem,
    *, n_pairs, head_dim, win, win_start,
):
    T, G, lag = _T, _GROUPS, _LAG
    f32, bf16 = jnp.float32, jnp.bfloat16
    scale = head_dim ** -0.5
    rows = 2 * head_dim
    nb = rows // T
    d_model = wq_v.shape[0]
    ncol = win // T
    gcols = ncol // G
    gw = gcols * T
    per = gcols * nb
    n_per = n_pairs * G
    assert lag <= per
    k_timer = kbuf.at[n_pairs * rows:, 0:T]
    v_timer = vbuf.at[rows:, 0:T]

    def piece(src, dst, dst_row0, c, g, i):
        r = (i % nb) * T
        col = _aligned(g * gw + (i // nb) * T, T)
        return pltpu.make_async_copy(
            src.at[pl.ds(_aligned(c * rows + r, T), T), pl.ds(win_start + col, T)],
            dst.at[pl.ds(_aligned(dst_row0 + r, T), T), pl.ds(col, T)], psem.at[g])

    def k_piece(p, i):
        p = p + i // per
        c = p // G
        return piece(kt_hbm, kbuf, c * rows, c, p % G, i % per)

    def v_piece(c, g, i):
        g = g + i // per
        return piece(vt_hbm, vbuf, 0, c + g // G, g % G, i % per)

    def group_wait(buf, row0, g):
        dst = buf.at[pl.ds(_aligned(row0, T), rows), pl.ds(_aligned(g * gw, gw), gw)]
        pltpu.make_async_copy(dst, dst, psem.at[g]).wait()

    def k_wait(p):
        group_wait(kbuf, (p // G) * rows, p % G)

    x_copy = pltpu.make_async_copy(x_hbm, x_v, wsem.at[0])
    wq_copy = pltpu.make_async_copy(wq_hbm, wq_v, wsem.at[1])
    wo_copy = pltpu.make_async_copy(wo_hbm, wo_v, wsem.at[2])
    w1_copy = pltpu.make_async_copy(w1_hbm, w1_v, wsem.at[3])
    w3_copy = pltpu.make_async_copy(w3_hbm, w3_v, wsem.at[4])
    offs = [0]
    for n in _W2_SPLIT:
        offs.append(offs[-1] + n)
    w2_copies = [
        pltpu.make_async_copy(w2_hbm.at[pl.ds(offs[i], n), :],
                              w2_v.at[pl.ds(offs[i], n), :], wsem.at[5 + i])
        for i, n in enumerate(_W2_SPLIT)]
    late_copies = [w1_copy, w3_copy] + w2_copies

    def slots(lo, hi, start_fn, items, ticks, timer_of):
        deps = {}
        for i in range(lo, hi):
            start_fn(i + lag)
            t = timer_of(i)[...].astype(f32)[0:8]
            n_ops = ticks
            if i in deps:
                t = t + functools.reduce(lambda a, b: a + b, deps[i])
                n_ops -= 1
            for e in range(n_ops):
                t = t * 0.5 if e % 2 == 0 else t + 0.25
            for item in items.get(i, []):
                r = item()
                if r is not None:
                    deps.setdefault(i + _DEP_LAG, []).append(r)
            timer_of(i + 1)[...] = jnp.concatenate([t, t], axis=0).astype(bf16)

    def k_slots(lo, hi, start_fn, items):
        slots(lo, hi, start_fn, items, _K_TICKS, lambda i: k_timer)

    wq_copy.start(priority=1)
    x_copy.start()
    k_timer[...] = jnp.zeros((16, T), bf16)
    k_slots(-lag, -7, lambda i: k_piece(0, i).start(), {})
    x_copy.wait()
    xn = _layernorm_f32(x_v[...].astype(f32)).astype(bf16)
    xn_s[...] = jnp.broadcast_to(xn, (8, d_model))
    k_slots(-7, 0, lambda i: k_piece(0, i).start(), {})

    def k_period(p, carry):
        @pl.when(p == _WO_AT)
        def _():
            wo_copy.start(priority=1)

        @pl.when(p > 0)
        def _():
            k_wait(p - 1)

        k_slots(0, per, lambda i: k_piece(p, i).start(), {})
        return carry

    jax.lax.fori_loop(0, n_per - 1, k_period, 0)

    row_id = jax.lax.broadcasted_iota(jnp.int32, (8, rows), 0)
    col_id = jax.lax.broadcasted_iota(jnp.int32, (8, rows), 1)
    diag = jnp.logical_and(col_id >= row_id * head_dim,
                           col_id < (row_id + 1) * head_dim)

    def q_items(items, c):
        for k in range(nb):
            def item(k=k):
                q = jnp.dot(xn_s[...], wq_v[:, pl.ds(_aligned(c * rows + k * T, T), T)],
                            preferred_element_type=f32)
                q_s[:, k * T:(k + 1) * T] = jnp.where(
                    diag[:, k * T:(k + 1) * T], q, 0.0).astype(bf16)
                return q
            items.setdefault(2 * k, []).append(item)

    def qk_items(items, c, cols, lo, hi):
        for i, slot in zip(cols, _spread(len(cols), lo, hi)):
            def item(i=i):
                s = jnp.dot(
                    q_s[...], kbuf[pl.ds(_aligned(c * rows, T), rows), i * T:(i + 1) * T],
                    preferred_element_type=f32)
                s_scr[:, i * T:(i + 1) * T] = s
                return s
            items.setdefault(slot, []).append(item)

    cuts = (0,) + tuple(_QK_SPLIT) + (ncol,)
    head = per - lag
    k_wait(n_per - 2)
    wq_copy.wait()
    items = {}
    q_items(items, 0)
    qk_items(items, 0, range(cuts[G - 1]), _Q_SLOTS, _MXU_HI)
    slots(0, per,
          lambda i: (k_piece(n_per - 1, i) if i < per else v_piece(0, 0, i - per)).start(),
          items, _K_TICKS, lambda i: k_timer if i < head else v_timer)

    nt_dims = (((1,), (1,)), ((), ()))

    def pv_tile(pslot, g, i):
        c0 = g * gw + (i // nb) * T
        r0 = (i % nb) * T
        return jax.lax.dot_general(p_scr[pslot, :, c0:c0 + T], vbuf[r0:r0 + T, c0:c0 + T],
                                   nt_dims, preferred_element_type=f32)

    def o_pair(parts, linv):
        o = jnp.concatenate(parts, axis=1)
        return jnp.where(diag, o * linv, 0.0).astype(bf16)

    def pair_body(c, linv_prev):
        st = {}
        c_next = jnp.minimum(c + 1, n_pairs - 1)

        def pv_items(items, acc, pslot, g, tiles, lo, hi):
            for i, slot in zip(tiles, _spread(len(tiles), lo, hi)):
                def item(i=i):
                    o = pv_tile(pslot, g, i)
                    acc[i % nb] = o if acc[i % nb] is None else acc[i % nb] + o
                    return o
                items.setdefault(slot, []).append(item)

        def softmax():
            s = s_scr[...]
            m = jnp.max(s, axis=-1, keepdims=True)
            p = jnp.exp((s - m) * scale)
            st["linv"] = 1.0 / jnp.sum(p, axis=-1, keepdims=True)
            p_scr[c % 2] = p.astype(bf16)

        def save(acc):
            for k in range(nb):
                oacc[k] = acc[k]

        def background():
            for j, cp in enumerate(late_copies):
                @pl.when(c == j)
                def _():
                    cp.start(priority=1)

        acc = [None] * nb
        for g in range(G):
            def v_slots(lo, hi, items, g=g):
                slots(lo, hi, lambda i: v_piece(c, g, i).start(), items, _V_TICKS,
                      lambda i: v_timer)

            items = {}
            if g == 0:
                @pl.when(c == 0)
                def _():
                    k_wait(n_per - 1)

                @pl.when(c > 0)
                def _():
                    group_wait(vbuf, 0, G - 1)

                prev = [oacc[k] for k in range(nb)]
                pv_items(items, prev, (c + 1) % 2, G - 1, range(per), 0, _MXU_HI)

                def finish():
                    o_s[c] = o_pair(prev, linv_prev)
                items.setdefault(_MXU_HI, []).append(finish)
                qk_items(items, c, range(cuts[G - 1], ncol), 0, _QK_HI)
                items.setdefault(_QK_HI + 1, []).append(softmax)
                v_slots(0, per, items)
                continue
            group_wait(vbuf, 0, g - 1)
            if g < G - 1:
                if g == 1:
                    q_items(items, c_next)
                else:
                    items[_MXU_HI] = [background]
                pv_items(items, acc, c % 2, g - 1, range(per), 0, _MXU_HI)
                qk_items(items, c_next, range(cuts[g - 1], cuts[g]),
                         _Q_SLOTS if g == 1 else 0, _MXU_HI)
                v_slots(0, per, items)
                continue
            pv_items(items, acc, c % 2, g - 1, range(_HEAD_TILES), 0, head - 3)
            v_slots(0, head, items)

            @pl.when(c < n_pairs - 1)
            def _():
                items, acc2 = {}, list(acc)
                pv_items(items, acc2, c % 2, g - 1, range(_HEAD_TILES, per), head, _MXU_HI)
                qk_items(items, c + 1, range(cuts[g - 1], cuts[g]), head, _MXU_HI)
                v_slots(head, per, items)
                save(acc2)

            @pl.when(c == n_pairs - 1)
            def _():
                acc2 = list(acc)
                for i in range(_HEAD_TILES, per):
                    acc2[i % nb] = acc2[i % nb] + pv_tile(c % 2, g - 1, i)
                save(acc2)
        return st["linv"]

    linv = jax.lax.fori_loop(0, n_pairs, pair_body, jnp.ones((8, 1), f32))

    wo_copy.wait()
    acc = jnp.zeros((8, d_model), f32)
    for c in range(n_pairs - 1):
        acc = acc + jnp.dot(o_s[c + 1], wo_v[c * rows:(c + 1) * rows, :],
                            preferred_element_type=f32)
    group_wait(vbuf, 0, G - 1)
    last = [oacc[k] for k in range(nb)]
    for i in range(per):
        last[i % nb] = last[i % nb] + pv_tile((n_pairs - 1) % 2, G - 1, i)
    acc = acc + jnp.dot(o_pair(last, linv), wo_v[(n_pairs - 1) * rows:, :],
                        preferred_element_type=f32)
    h = x_v[...].astype(f32) + jnp.sum(acc, axis=0, keepdims=True)

    hn8 = jnp.broadcast_to(_layernorm_f32(h).astype(bf16), (8, d_model))
    w1_copy.wait()
    w3_copy.wait()
    gate = jnp.dot(hn8, w1_v[...], preferred_element_type=f32)
    up = jnp.dot(hn8, w3_v[...], preferred_element_type=f32)
    act = (gate * jax.nn.sigmoid(gate) * up).astype(bf16)
    res = jnp.broadcast_to(h, (8, d_model))
    for i in range(len(w2_copies) - 1):
        w2_copies[i].wait()
        if i == 0:
            col = jnp.broadcast_to(act[0:1, offs[-1] - T:].astype(f32), (T, T)).T
            col = col[T - _W2_SPLIT[-1]:, :]
        res = res + jnp.dot(act[:, offs[i]:offs[i + 1]], w2_v[offs[i]:offs[i + 1], :],
                            preferred_element_type=f32)
    w2_copies[-1].wait()
    w_last = w2_v[offs[-2]:offs[-1], :].astype(f32)
    prod = w_last * jnp.concatenate([col] * (d_model // T), axis=1)
    o_ref[...] = (res[0:1, :] + jnp.sum(prod, axis=0, keepdims=True)).astype(o_ref.dtype)


@jax.jit
def pallas_sequential_preLN__sliding_block_cached__glu_gated_swiglu__decode_kernel(
    A_x: jax.Array,
    A_k_cache: jax.Array,
    A_v_cache: jax.Array,
    A_wq: jax.Array,
    A_wo: jax.Array,
    B_x: jax.Array,
    B_w1: jax.Array,
    B_w3: jax.Array,
    B_w2: jax.Array,
):
    B, Sq, D = A_x.shape
    _, H, Sk, Dh = A_k_cache.shape
    F = B_w1.shape[1]
    W = min(4096, max(256, Sk // 4))
    assert B == 1 and Sq == 1 and H % 2 == 0 and 2 * Dh == 3 * _T
    assert sum(_W2_SPLIT) == F and W == 32 * _T and (Sk - W) % _T == 0

    kt = jnp.swapaxes(A_k_cache, 2, 3).reshape(H * Dh, Sk)
    vt = jnp.swapaxes(A_v_cache, 2, 3).reshape(H * Dh, Sk)
    x2 = A_x.reshape(1, D)

    params = dict(vmem_limit_bytes=100 * 1024 * 1024)
    for name in ("disable_semaphore_checks", "disable_bounds_checks"):
        if hasattr(pltpu.CompilerParams, name):
            params[name] = True

    bf16 = jnp.bfloat16
    out = pl.pallas_call(
        functools.partial(_kernel, n_pairs=H // 2, head_dim=Dh, win=W, win_start=Sk - W),
        out_shape=jax.ShapeDtypeStruct((1, D), A_x.dtype),
        in_specs=[pl.BlockSpec(memory_space=pl.ANY)] * 8,
        out_specs=pl.BlockSpec(memory_space=pltpu.VMEM),
        scratch_shapes=[
            pltpu.VMEM((1, D), bf16),
            pltpu.VMEM((H * Dh + 16, W), bf16),
            pltpu.VMEM((2 * Dh + 16, W), bf16),
            pltpu.VMEM((D, H * Dh), bf16),
            pltpu.VMEM((H * Dh, D), bf16),
            pltpu.VMEM((D, F), bf16),
            pltpu.VMEM((D, F), bf16),
            pltpu.VMEM((F, D), bf16),
            pltpu.VMEM((8, D), bf16),
            pltpu.VMEM((8, 2 * Dh), bf16),
            pltpu.VMEM((8, W), jnp.float32),
            pltpu.VMEM((2, 8, W), bf16),
            pltpu.VMEM((2 * Dh // _T, 8, _T), jnp.float32),
            pltpu.VMEM((H // 2, 8, 2 * Dh), bf16),
            pltpu.SemaphoreType.DMA((_GROUPS,)),
            pltpu.SemaphoreType.DMA((5 + len(_W2_SPLIT),)),
        ],
        compiler_params=pltpu.CompilerParams(**params),
    )(x2, kt, vt, A_wq, A_wo, B_w1, B_w3, B_w2)
    return out.reshape(B, Sq, D)
```

```python
import functools

import jax
import jax.numpy as jnp
import jax.experimental.pallas as pl
import jax.experimental.pallas.tpu as pltpu

_EPS = 1e-5
_T = 128
_GROUPS = 4
_LAG = 18
_K_TICKS = 29
_V_TICKS = 28
_DEP_LAG = 4
_QK_SPLIT = (6, 15, 24)
_QK_HI = 13
_MXU_HI = 21
_Q_SLOTS = 9
_HEAD_TILES = 3
_WO_AT = 8
_W2_SPLIT = (1024, 384, 128)


def _layernorm_f32(x):
    m = jnp.mean(x, axis=-1, keepdims=True)
    c = x - m
    v = jnp.mean(c * c, axis=-1, keepdims=True)
    return c / jnp.sqrt(v + _EPS)


def _spread(n_items, lo, hi):
    return [lo + (t * (hi - lo)) // n_items for t in range(n_items)]


def _aligned(v, m):
    return v if isinstance(v, int) else pl.multiple_of(v, m)


def _kernel(
    x_hbm, kt_hbm, vt_hbm, wq_hbm, wo_hbm, w1_hbm, w3_hbm, w2_hbm,
    o_ref,
    x_v, kbuf, vbuf, wq_v, wo_v, w1_v, w3_v, w2_v, xn_s, q_s, s_scr, p_scr, linv_s, oacc, o_s,
    psem, wsem,
    *, n_pairs, head_dim, win, win_start,
):
    T, G, lag = _T, _GROUPS, _LAG
    f32, bf16 = jnp.float32, jnp.bfloat16
    scale = head_dim ** -0.5
    rows = 2 * head_dim
    nb = rows // T
    d_model = wq_v.shape[0]
    ncol = win // T
    gcols = ncol // G
    gw = gcols * T
    per = gcols * nb
    n_per = n_pairs * G
    assert lag <= per
    k_timer = kbuf.at[n_pairs * rows:, 0:T]
    v_timer = vbuf.at[rows:, 0:T]

    def piece(src, dst, dst_row0, c, g, i):
        r = (i % nb) * T
        col = _aligned(g * gw + (i // nb) * T, T)
        return pltpu.make_async_copy(
            src.at[pl.ds(_aligned(c * rows + r, T), T), pl.ds(win_start + col, T)],
            dst.at[pl.ds(_aligned(dst_row0 + r, T), T), pl.ds(col, T)], psem.at[g])

    def k_piece(p, i):
        p = p + i // per
        c = p // G
        return piece(kt_hbm, kbuf, c * rows, c, p % G, i % per)

    def v_piece(c, g, i):
        g = g + i // per
        return piece(vt_hbm, vbuf, 0, c + g // G, g % G, i % per)

    def group_wait(buf, row0, g):
        dst = buf.at[pl.ds(_aligned(row0, T), rows), pl.ds(_aligned(g * gw, gw), gw)]
        pltpu.make_async_copy(dst, dst, psem.at[g]).wait()

    def k_wait(p):
        group_wait(kbuf, (p // G) * rows, p % G)

    x_copy = pltpu.make_async_copy(x_hbm, x_v, wsem.at[0])
    wq_copy = pltpu.make_async_copy(wq_hbm, wq_v, wsem.at[1])
    wo_copy = pltpu.make_async_copy(wo_hbm, wo_v, wsem.at[2])
    w1_copy = pltpu.make_async_copy(w1_hbm, w1_v, wsem.at[3])
    w3_copy = pltpu.make_async_copy(w3_hbm, w3_v, wsem.at[4])
    offs = [0]
    for n in _W2_SPLIT:
        offs.append(offs[-1] + n)
    w2_copies = [
        pltpu.make_async_copy(w2_hbm.at[pl.ds(offs[i], n), :],
                              w2_v.at[pl.ds(offs[i], n), :], wsem.at[5 + i])
        for i, n in enumerate(_W2_SPLIT)]
    late_copies = [w1_copy, w3_copy] + w2_copies

    def slots(lo, hi, start_fn, items, ticks, timer_of):
        deps = {}
        for i in range(lo, hi):
            start_fn(i + lag)
            t = timer_of(i)[...].astype(f32)[0:8]
            n_ops = ticks
            if i in deps:
                t = t + functools.reduce(lambda a, b: a + b, deps[i])
                n_ops -= 1
            for e in range(n_ops):
                t = t * 0.5 if e % 2 == 0 else t + 0.25
            for item in items.get(i, []):
                r = item()
                if r is not None:
                    deps.setdefault(i + _DEP_LAG, []).append(r)
            timer_of(i + 1)[...] = jnp.concatenate([t, t], axis=0).astype(bf16)

    def k_slots(lo, hi, start_fn, items):
        slots(lo, hi, start_fn, items, _K_TICKS, lambda i: k_timer)

    wq_copy.start(priority=1)
    x_copy.start()
    k_timer[...] = jnp.zeros((16, T), bf16)
    k_slots(-lag, -7, lambda i: k_piece(0, i).start(), {})
    x_copy.wait()
    xn = _layernorm_f32(x_v[...].astype(f32)).astype(bf16)
    xn_s[...] = jnp.broadcast_to(xn, (8, d_model))
    k_slots(-7, 0, lambda i: k_piece(0, i).start(), {})

    def k_period(p, carry):
        @pl.when(p == _WO_AT)
        def _():
            wo_copy.start(priority=1)

        @pl.when(p > 0)
        def _():
            k_wait(p - 1)

        k_slots(0, per, lambda i: k_piece(p, i).start(), {})
        return carry

    jax.lax.fori_loop(0, n_per - 1, k_period, 0)

    row_id = jax.lax.broadcasted_iota(jnp.int32, (8, rows), 0)
    col_id = jax.lax.broadcasted_iota(jnp.int32, (8, rows), 1)
    diag = jnp.logical_and(col_id >= row_id * head_dim,
                           col_id < (row_id + 1) * head_dim)

    def q_items(items, c):
        for k in range(nb):
            def item(k=k):
                q = jnp.dot(xn_s[...], wq_v[:, pl.ds(_aligned(c * rows + k * T, T), T)],
                            preferred_element_type=f32)
                q_s[:, k * T:(k + 1) * T] = jnp.where(
                    diag[:, k * T:(k + 1) * T], q, 0.0).astype(bf16)
                return q
            items.setdefault(2 * k, []).append(item)

    def qk_items(items, c, cols, lo, hi):
        for i, slot in zip(cols, _spread(len(cols), lo, hi)):
            def item(i=i):
                s = jnp.dot(
                    q_s[...], kbuf[pl.ds(_aligned(c * rows, T), rows), i * T:(i + 1) * T],
                    preferred_element_type=f32)
                s_scr[:, i * T:(i + 1) * T] = s
                return s
            items.setdefault(slot, []).append(item)

    cuts = (0,) + tuple(_QK_SPLIT) + (ncol,)
    head = per - lag
    k_wait(n_per - 2)
    wq_copy.wait()
    items = {}
    q_items(items, 0)
    qk_items(items, 0, range(cuts[G - 1]), _Q_SLOTS, _MXU_HI)
    slots(0, per,
          lambda i: (k_piece(n_per - 1, i) if i < per else v_piece(0, 0, i - per)).start(),
          items, _K_TICKS, lambda i: k_timer if i < head else v_timer)

    nt_dims = (((1,), (1,)), ((), ()))

    def pv_tile(pslot, g, i):
        c0 = g * gw + (i // nb) * T
        r0 = (i % nb) * T
        return jax.lax.dot_general(p_scr[pslot, :, c0:c0 + T], vbuf[r0:r0 + T, c0:c0 + T],
                                   nt_dims, preferred_element_type=f32)

    def o_pair(parts, linv):
        o = jnp.concatenate(parts, axis=1)
        return jnp.where(diag, o * linv, 0.0).astype(bf16)

    def v_slots(c, g, lo, hi, items):
        slots(lo, hi, lambda i: v_piece(c, g, i).start(), items, _V_TICKS,
              lambda i: v_timer)

    def pv_items(items, acc, pslot, g, tiles, lo, hi):
        for i, slot in zip(tiles, _spread(len(tiles), lo, hi)):
            def item(i=i):
                o = pv_tile(pslot, g, i)
                acc[i % nb] = o if acc[i % nb] is None else acc[i % nb] + o
                return o
            items.setdefault(slot, []).append(item)

    def score_items(items, c):
        def softmax():
            s = s_scr[...]
            m = jnp.max(s, axis=-1, keepdims=True)
            p = jnp.exp((s - m) * scale)
            linv_s[c % 2] = 1.0 / jnp.sum(p, axis=-1, keepdims=True)
            p_scr[c % 2] = p.astype(bf16)

        qk_items(items, c, range(cuts[G - 1], ncol), 0, _QK_HI)
        items.setdefault(_QK_HI + 1, []).append(softmax)

    k_wait(n_per - 1)
    items = {}
    score_items(items, 0)
    v_slots(0, 0, 0, per, items)

    def pair_body(c, carry):
        c_next = jnp.minimum(c + 1, n_pairs - 1)
        pslot = c % 2

        def background():
            for j, cp in enumerate(late_copies):
                @pl.when(c == j)
                def _():
                    cp.start(priority=1)

        acc = [None] * nb
        for g in range(1, G - 1):
            group_wait(vbuf, 0, g - 1)
            items = {}
            if g == 1:
                q_items(items, c_next)
            else:
                items[_MXU_HI] = [background]
            pv_items(items, acc, pslot, g - 1, range(per), 0, _MXU_HI)
            qk_items(items, c_next, range(cuts[g - 1], cuts[g]),
                     _Q_SLOTS if g == 1 else 0, _MXU_HI)
            v_slots(c, g, 0, per, items)

        g = G - 1
        group_wait(vbuf, 0, g - 1)
        items = {}
        pv_items(items, acc, pslot, g - 1, range(_HEAD_TILES), 0, head - 3)
        v_slots(c, g, 0, head, items)

        @pl.when(c < n_pairs - 1)
        def _():
            items, acc2 = {}, list(acc)
            pv_items(items, acc2, pslot, g - 1, range(_HEAD_TILES, per), head, _MXU_HI)
            qk_items(items, c + 1, range(cuts[g - 1], cuts[g]), head, _MXU_HI)
            v_slots(c, g, head, per, items)

            def finish():
                o_s[c] = o_pair(acc2, linv_s[pslot])

            group_wait(vbuf, 0, g)
            items = {_MXU_HI: [finish]}
            pv_items(items, acc2, pslot, g, range(per), 0, _MXU_HI)
            score_items(items, c + 1)
            v_slots(c + 1, 0, 0, per, items)

        @pl.when(c == n_pairs - 1)
        def _():
            acc2 = list(acc)
            for i in range(_HEAD_TILES, per):
                acc2[i % nb] = acc2[i % nb] + pv_tile(pslot, g - 1, i)
            for k in range(nb):
                oacc[k] = acc2[k]
        return carry

    jax.lax.fori_loop(0, n_pairs, pair_body, 0)

    wo_copy.wait()
    acc = jnp.zeros((8, d_model), f32)
    for c in range(n_pairs - 1):
        acc = acc + jnp.dot(o_s[c], wo_v[c * rows:(c + 1) * rows, :],
                            preferred_element_type=f32)
    group_wait(vbuf, 0, G - 1)
    pslot = (n_pairs - 1) % 2
    last = [oacc[k] for k in range(nb)]
    for i in range(per):
        last[i % nb] = last[i % nb] + pv_tile(pslot, G - 1, i)
    acc = acc + jnp.dot(o_pair(last, linv_s[pslot]), wo_v[(n_pairs - 1) * rows:, :],
                        preferred_element_type=f32)
    h = x_v[...].astype(f32) + jnp.sum(acc, axis=0, keepdims=True)

    hn8 = jnp.broadcast_to(_layernorm_f32(h).astype(bf16), (8, d_model))
    w1_copy.wait()
    w3_copy.wait()
    gate = jnp.dot(hn8, w1_v[...], preferred_element_type=f32)
    up = jnp.dot(hn8, w3_v[...], preferred_element_type=f32)
    act = (gate * jax.nn.sigmoid(gate) * up).astype(bf16)
    res = jnp.broadcast_to(h, (8, d_model))
    for i in range(len(w2_copies) - 1):
        w2_copies[i].wait()
        if i == 0:
            col = jnp.broadcast_to(act[0:1, offs[-1] - T:].astype(f32), (T, T)).T
            col = col[T - _W2_SPLIT[-1]:, :]
        res = res + jnp.dot(act[:, offs[i]:offs[i + 1]], w2_v[offs[i]:offs[i + 1], :],
                            preferred_element_type=f32)
    w2_copies[-1].wait()
    w_last = w2_v[offs[-2]:offs[-1], :].astype(f32)
    prod = w_last * jnp.concatenate([col] * (d_model // T), axis=1)
    o_ref[...] = (res[0:1, :] + jnp.sum(prod, axis=0, keepdims=True)).astype(o_ref.dtype)


@jax.jit
def pallas_sequential_preLN__sliding_block_cached__glu_gated_swiglu__decode_kernel(
    A_x: jax.Array,
    A_k_cache: jax.Array,
    A_v_cache: jax.Array,
    A_wq: jax.Array,
    A_wo: jax.Array,
    B_x: jax.Array,
    B_w1: jax.Array,
    B_w3: jax.Array,
    B_w2: jax.Array,
):
    B, Sq, D = A_x.shape
    _, H, Sk, Dh = A_k_cache.shape
    F = B_w1.shape[1]
    W = min(4096, max(256, Sk // 4))
    assert B == 1 and Sq == 1 and H % 2 == 0 and 2 * Dh == 3 * _T
    assert sum(_W2_SPLIT) == F and W == 32 * _T and (Sk - W) % _T == 0

    kt = jnp.swapaxes(A_k_cache, 2, 3).reshape(H * Dh, Sk)
    vt = jnp.swapaxes(A_v_cache, 2, 3).reshape(H * Dh, Sk)
    x2 = A_x.reshape(1, D)

    params = dict(vmem_limit_bytes=100 * 1024 * 1024)
    for name in ("disable_semaphore_checks", "disable_bounds_checks"):
        if hasattr(pltpu.CompilerParams, name):
            params[name] = True

    bf16 = jnp.bfloat16
    out = pl.pallas_call(
        functools.partial(_kernel, n_pairs=H // 2, head_dim=Dh, win=W, win_start=Sk - W),
        out_shape=jax.ShapeDtypeStruct((1, D), A_x.dtype),
        in_specs=[pl.BlockSpec(memory_space=pl.ANY)] * 8,
        out_specs=pl.BlockSpec(memory_space=pltpu.VMEM),
        scratch_shapes=[
            pltpu.VMEM((1, D), bf16),
            pltpu.VMEM((H * Dh + 16, W), bf16),
            pltpu.VMEM((2 * Dh + 16, W), bf16),
            pltpu.VMEM((D, H * Dh), bf16),
            pltpu.VMEM((H * Dh, D), bf16),
            pltpu.VMEM((D, F), bf16),
            pltpu.VMEM((D, F), bf16),
            pltpu.VMEM((F, D), bf16),
            pltpu.VMEM((8, D), bf16),
            pltpu.VMEM((8, 2 * Dh), bf16),
            pltpu.VMEM((8, W), jnp.float32),
            pltpu.VMEM((2, 8, W), bf16),
            pltpu.VMEM((2, 8, 1), jnp.float32),
            pltpu.VMEM((2 * Dh // _T, 8, _T), jnp.float32),
            pltpu.VMEM((H // 2 - 1, 8, 2 * Dh), bf16),
            pltpu.SemaphoreType.DMA((_GROUPS,)),
            pltpu.SemaphoreType.DMA((5 + len(_W2_SPLIT),)),
        ],
        compiler_params=pltpu.CompilerParams(**params),
    )(x2, kt, vt, A_wq, A_wo, B_w1, B_w3, B_w2)
    return out.reshape(B, Sq, D)
```
